```python
import jax
import jax.numpy as jnp

def _softmax(x, axis=-1):
    return jax.nn.softmax(x, axis=axis)

def _gelu(x):
    return jax.nn.gelu(x, approximate=True)

def _silu(x):
    return jax.nn.silu(x)

def _sigmoid(x):
    return jax.nn.sigmoid(x)

def _layernorm(x, axis=-1, eps=1e-05):
    m = jnp.mean(x, axis=axis, keepdims=True)
    v = jnp.var(x, axis=axis, keepdims=True)
    return (x - m) / jnp.sqrt(v + eps)

def _scatter_add(tgt, idx, src, axis=0):
    return tgt.at[idx].add(src)

def _segment_sum(src, seg, n):
    return jax.ops.segment_sum(src, seg, n)

class _Rng:

    def __init__(self, key):
        self._k = key

    def _next(self):
        self._k, sub = jax.random.split(self._k)
        return sub

    def normal(self, shape):
        return jax.random.normal(self._next(), shape, dtype=jnp.bfloat16)

    def randint(self, lo, hi, shape):
        return jax.random.randint(self._next(), shape, lo, hi, dtype=jnp.int32)

    def uniform(self, shape, lo=0.0, hi=1.0):
        return jax.random.uniform(self._next(), shape, jnp.bfloat16, lo, hi)

    def permutation(self, n):
        return jax.random.permutation(self._next(), n)
kernel_name = 'adaLN_cond__grouped_kv_mqa__dense_activation_silu__prompt'

def _fwd_setup_inputs():
    _rng = _Rng(jax.random.key(int.from_bytes(__import__("os").urandom(4), "little")))
    _w = lambda a: (lambda t: t.astype(jnp.bfloat16) if jnp.issubdtype(t.dtype, jnp.floating) else t)(jnp.asarray(a))

    def _A_setup():
        B, S, D, H = (1, 2048, 640, 32)
        Dh = D // H
        return {'x': _w((lambda *s: _rng.normal(s) * 0.05)(B, S, D)), 'wq': _w((lambda *s: _rng.normal(s) * 0.05)(D, H * Dh)), 'wk': _w((lambda *s: _rng.normal(s) * 0.05)(D, Dh)), 'wv': _w((lambda *s: _rng.normal(s) * 0.05)(D, Dh)), 'wo': _w((lambda *s: _rng.normal(s) * 0.05)(H * Dh, D))}
    _A_in = _A_setup()

    def _B_setup():
        B, S, D, F = (1, 2048, 640, 1728)
        return {'x': _w((lambda *s: _rng.normal(s) * 0.05)(B, S, D)), 'w1': _w((lambda *s: _rng.normal(s) * 0.05)(D, F) * D ** (-0.5)), 'w2': _w((lambda *s: _rng.normal(s) * 0.05)(F, D) * F ** (-0.5))}
    _B_in = _B_setup()
    return {'A_x': _A_in['x'], 'A_wq': _A_in['wq'], 'A_wk': _A_in['wk'], 'A_wv': _A_in['wv'], 'A_wo': _A_in['wo'], 'B_x': _B_in['x'], 'B_w1': _B_in['w1'], 'B_w2': _B_in['w2'], 'c': _w((lambda *s: _rng.normal(s) * 0.05)(1, 640)), 'w_mod': _w((lambda *s: _rng.normal(s) * 0.05)(640, 6 * 640) * 640 ** (-0.5))}

def _fwd_reference(A_x, A_wq, A_wk, A_wv, A_wo, B_x, B_w1, B_w2, c, w_mod):

    def _A_ref(x, wq, wk, wv, wo):
        B, S, D = x.shape
        H = 32
        Dh = D // H
        q = (lambda x, *d: x.transpose(*d))((x @ wq).reshape(B, S, H, Dh), 0, 2, 1, 3)
        k = x @ wk
        v = x @ wv
        scores = jnp.einsum('bhqd,bkd->bhqk', q, k) * Dh ** (-0.5)
        p = _softmax(scores, axis=-1)
        o = jnp.einsum('bhqk,bkd->bhqd', p, v)
        return (lambda x, *d: x.transpose(*d))(o, 0, 2, 1, 3).reshape(B, S, H * Dh) @ wo

    def _B_ref(x, w1, w2):
        h = jnp.einsum('bsd,df->bsf', x, w1)
        h = _silu(h)
        out = jnp.einsum('bsf,fd->bsd', h, w2)
        return out
    x = A_x
    mod = (_silu(c) @ w_mod).reshape(c.shape[0], 6, 1, -1)
    sa, ca, ga, sb, cb, gb = (mod[:, 0].copy(), mod[:, 1].copy(), mod[:, 2].copy(), mod[:, 3].copy(), mod[:, 4].copy(), mod[:, 5].copy())
    h = _layernorm(x, axis=-1) * (1 + ca) + sa
    x = x + ga * _A_ref(h, A_wq, A_wk, A_wv, A_wo)
    h = _layernorm(x, axis=-1) * (1 + cb) + sb
    x = x + gb * _B_ref(h, B_w1, B_w2)
    return x

def setup_inputs():
    _inp = _fwd_setup_inputs()
    _gk = jax.random.fold_in(jax.random.key(int.from_bytes(__import__("os").urandom(4), "little")), 2 ** 31 - 1)
    _shapes = [[1, 2048, 640]]
    _dtypes = ['bfloat16']
    _gks = jax.random.split(_gk, len(_shapes))
    _gs = [jax.random.normal(k, s, dtype=jnp.dtype(d)) * 0.05 for k, s, d in zip(_gks, _shapes, _dtypes)]
    _inp['grad_out'] = _gs[0]
    return _inp

def reference(A_x, A_wq, A_wk, A_wv, A_wo, B_w1, B_w2, c, w_mod, B_x, grad_out):
    _const = dict(B_x=B_x)

    def _f(*_d):
        return _fwd_reference(**{'A_x': _d[0], 'A_wq': _d[1], 'A_wk': _d[2], 'A_wv': _d[3], 'A_wo': _d[4], 'B_w1': _d[5], 'B_w2': _d[6], 'c': _d[7], 'w_mod': _d[8], **_const})
    _out, _vjp = jax.vjp(_f, A_x, A_wq, A_wk, A_wv, A_wo, B_w1, B_w2, c, w_mod)
    _grads = _vjp(grad_out)
    _out0 = jnp.asarray(_out)
    return (_out0, *[jnp.asarray(_g) for _g in _grads])
```

```python
import functools
import math

import jax
import jax.numpy as jnp
from jax import lax
import jax.experimental.pallas as pl
import jax.experimental.pallas.tpu as pltpu

f32, bf16 = jnp.float32, jnp.bfloat16

S, D, H, F = 2048, 640, 32, 1728
DH = D // H
W = 24
WB = 32
TQ = 512
NB = S // TQ
KC = 128
NC = S // KC
HF = 8
HU = 4
LAG = 1
PACE = 3
K_GROUPS = (120, 248, 376, 504, 496)
V_GROUPS = (0, 128, 256, 384)
FC = 144
DC = 160
MC = 80
FH, TH, MH = F // 2, TQ // 2, D // 2
D1, D2 = 384, 256
KT = -(-FH // 128)
EPS = 1e-5
SCALE = DH ** -0.5
LOG2E = math.log2(math.e)
GATE_A, SHIFT_B, SCALE_B, GATE_B = range(4)

_NN = (((1,), (0,)), ((), ()))
_NT = (((1,), (1,)), ((), ()))


def _nn(a, b):
    return lax.dot_general(a, b, _NN, preferred_element_type=f32)


def _nt(a, b):
    return lax.dot_general(a, b, _NT, preferred_element_type=f32)


def _round(x):
    return x.astype(bf16).astype(f32)


def _wide(col):
    return jnp.concatenate([col] * (TQ // 128), axis=1)


def _fold(x):
    out = x[:, :128]
    for j in range(1, TQ // 128):
        out = out + x[:, j * 128:(j + 1) * 128]
    return out


def _rows8(x):
    return jnp.sum(x.reshape(x.shape[0] // 8, 8, x.shape[1]), axis=0)


def _mean_rows(p):
    return jnp.sum(p, axis=0, keepdims=True) * (1.0 / D)


def _to_column(row):
    return jnp.broadcast_to(row, (128, D)).T


def _to_row(acc):
    return jnp.sum(acc.T, axis=0, keepdims=True)


def _pad_rhs(win):
    return jnp.concatenate(
        [win, jnp.zeros((WB - W, win.shape[1]), f32)], axis=0).astype(bf16)


def _spread(win):
    return [jnp.broadcast_to(win[d:d + 1], (8, TQ)) for d in range(DH)]


def _swap_pairs(x):
    return jnp.concatenate(
        [x[8 * (j ^ 1):8 * (j ^ 1) + 8] for j in range(x.shape[0] // 8)], axis=0)


def _chunks(n, size):
    return [slice(i * size, (i + 1) * size) for i in range(n // size)]


def _windows(group):
    pad = jnp.zeros((W - DH, group.shape[1]), f32)
    return [jnp.concatenate([group[u * DH:(u + 1) * DH], pad], axis=0)
            for u in range(group.shape[0] // DH)]


def _accumulate(total, term):
    return term if total is None else total + term


_RIGHT_AS_LEFT = (0, 2, 6, 5, 3, 4, 1)


def _left_combinations(a, b, c, d):
    return a + d, c + d, a, d, a + b, c - a, b - d


def _quadrants(m):
    return (m[3] - m[4] + m[0] + m[6], m[2] + m[4],
            m[1] + m[3], m[2] - m[1] + m[0] + m[5])


_SUM_ROWS = (0, D1, D1 + D2, 2 * D1 + D2, 2 * D1 + 2 * D2, 3 * D1 + 2 * D2)


def _store_sums(sums, raw):
    for r in _chunks(D1, 128):
        top = raw[r, :].astype(f32)
        a, c = top[:, :TH], top[:, TH:]
        if r.start < D2:
            bottom = raw[D1 + r.start:D1 + r.stop, :].astype(f32)
            b, d = bottom[:, :TH], bottom[:, TH:]
            parts = (a + d, b - d, c - a, a + b, c + d)
        else:
            parts = (a, None, c - a, None, c)
        for lo, part in zip(_SUM_ROWS, parts):
            if part is not None:
                sums[lo + r.start:lo + r.stop, :] = part.astype(bf16)


def _layer_norm_stats(chunks):
    means, m2 = [], None
    for x in chunks:
        x = x.reshape(x.shape[0] // 8, 8, x.shape[1])
        means.append(jnp.sum(x, axis=0) * (1.0 / x.shape[0]))
        xc = x - means[-1][None]
        m2 = _accumulate(m2, jnp.sum(xc * xc, axis=0))
    count = D // (8 * len(means))
    mu = _mean_rows(functools.reduce(jnp.add, means)) * count
    spread = functools.reduce(jnp.add, [(m - mu) * (m - mu) for m in means])
    return mu, lax.rsqrt(_mean_rows(m2 + spread * count) + EPS)


def _token_half(ref, i, rows):
    return jnp.concatenate([ref[2 * i, rows, :], ref[2 * i + 1, rows, :]], axis=1)


def _add_weight_grad(acc, fs, left, raw, sums):
    s = [sums[lo:hi, :] for lo, hi in zip(_SUM_ROWS, _SUM_ROWS[1:])]
    right = (s[0], raw[:D1, :TH], s[1], s[2], raw[D1:, TH:], s[3], s[4])
    m = [_nt(_token_half(left, i, fs), right[i]) for i in range(7)]
    f2 = slice(FH + fs.start, FH + fs.stop)
    acc[fs, :D2] += m[0][:, :D2] + m[3][:, :D2] - m[4] + m[6][:, :D2]
    acc[fs, D2:D1] += m[0][:, D2:] + m[3][:, D2:] + m[6][:, D2:]
    acc[fs, D1:] += m[2] + m[4]
    acc[f2, :D1] += m[1] + m[3]
    acc[f2, D1:] += m[0][:, :D2] - m[1][:, :D2] + m[2] + m[5]


def _down_projection(left, right):
    for r in _chunks(MH, MC):
        m = [None] * 7
        for i in (2, 4, 1, 3, 0, 5, 6):
            rows = slice(i * MH + r.start, i * MH + r.stop)
            lhs = [left[k, rows, :min(128, FH - k * 128)] for k in range(KT)]
            m[i] = _nn(jnp.concatenate(lhs, axis=1),
                       _token_half(right, _RIGHT_AS_LEFT[i], slice(None)))
        q = _quadrants(m)
        yield r, jnp.concatenate(q[:2], axis=1)
        yield slice(MH + r.start, MH + r.stop), jnp.concatenate(q[2:], axis=1)


def _kernel(*refs):
    shapes = [(NB, D, TQ), (NB, D, TQ), (NB * D, TQ),
              (TQ // 128, D, 128), (1, D, TQ), (D, TQ),
              (1, D, TQ), (1, D, TQ),
              (_SUM_ROWS[-1], TH), (_SUM_ROWS[-1], TH)]
    pl.run_scoped(functools.partial(_body, *refs), *[pltpu.VMEM(s, bf16) for s in shapes])


def _body(
    x_hbm, wq_hbm, wkT_hbm, wvT_hbm, wo_hbm, w1T_hbm, w2_hbm, c_hbm, wmod_hbm,
    dout_hbm,
    out_hbm, dx_hbm, dwq_hbm, dwkT_hbm, dwvT_hbm, dwo_hbm, dw1T_hbm, dw2_hbm,
    dc_hbm, dwmod_hbm,
    wkT, wvT, wo, woT, w1_left, w1T, w2, w2_left, c_v,
    modc, mod_rows, stat, ln1, kk, va, k_cols, v_cols, kT, vT, vT_swapped, dkT, dvT,
    s_buf, m_buf, ow, io_v, g_buf, du_buf,
    dwo_acc, dw1_acc, dw2_acc, dmod_v, zeros, sems,
    xT, dx1, qT, doT, dm_buf, oT, h2_buf, da_buf, h2_sums, dm_sums,
):
    dm, h2, da = dm_buf.at[0], h2_buf.at[0], da_buf.at[0]

    def copy(src, dst, i):
        return pltpu.make_async_copy(src, dst, sems.at[i])

    def tokens(b):
        return pl.ds(pl.multiple_of(b * TQ, TQ), TQ)

    def dout_copy(b):
        return copy(dout_hbm.at[tokens(b)], io_v, 16)

    def out_copy(b):
        return copy(io_v, out_hbm.at[tokens(b)], 17)

    def head_rows(h, n):
        return pl.ds(pl.multiple_of(h * DH, 4 * DH), n * DH)

    def key_tile(ref, kc):
        return ref.at[kc * KC // TQ, :, pl.ds(kc * KC % TQ, KC)]

    mod_stage = [(g_buf, du_buf)[i % 2].at[i // 2, pl.ds(0, D)] for i in range(4 * D // 128)]
    early_copies = [copy(wmod_hbm.at[:, pl.ds(2 * D + i * 128, 128)], ref, 18)
                    for i, ref in enumerate(mod_stage)]
    early_copies += [copy(wo_hbm, wo, 19), copy(w1T_hbm, w1T, 20), copy(w2_hbm, w2, 21)]
    wq_copy = copy(wq_hbm, wo, 22)
    grad_stage = [(w1_left, w2_left)[i % 2].at[i // 6, pl.ds(i // 2 % 3 * D, D)] for i in range(4 * D // 128)]
    grad_tiles = [(slice(half * FH, (half + 1) * FH), t) for half in range(2) for t in _chunks(D, 128)]
    grad_copies = [copy(src.at[i], dst.at[pl.ds(rows.start, FH), pl.ds(t.start, 128)], 28)
                   for i, (rows, t) in enumerate(grad_tiles)
                   for src, dst in ((du_buf, dw1T_hbm), (g_buf, dw2_hbm))]
    grad_copies += [copy(ref, dwmod_hbm.at[:, pl.ds(2 * D + i * 128, 128)], 28)
                    for i, ref in enumerate(grad_stage)]
    row_w = lax.broadcasted_iota(jnp.int32, (W, TQ), 0)

    def silu_c():
        cf = c_v[...].astype(f32)
        sg = jax.nn.sigmoid(cf)
        return cf * sg, sg * (1.0 + cf * (1.0 - sg))

    def set_modulation(dst, row, scale):
        for j, t in enumerate(_chunks(row.shape[1], D)):
            dst[j] = _to_column(row[:, t] + 1.0 if j == scale else row[:, t])

    def score_step(q, kc, slot, mx):
        weights, rows = q
        lanes, part = _chunks(TQ, 128)[kc // NB], kc % NB
        ks = slice(kc * KC, (kc + 1) * KC - 8 * sum(at // KC == part for at in K_GROUPS))
        s = _nn(kk[ks, :], weights)
        s_buf[slot, ks, :] = s
        rest = None
        for d in range(DH):
            rest = _accumulate(rest, k_cols[part, d] * jnp.concatenate(
                [rows[d][:, lanes]] * len(K_GROUPS), axis=0))
        for j, at in enumerate(K_GROUPS):
            s_buf[slot, part * TQ + at:part * TQ + at + 8, lanes] = rest[8 * j:8 * j + 8]
        parts = [jnp.concatenate([s[:104, t], rest, s[104:, t]], axis=0)
                 if t == lanes else s[:, t] for t in _chunks(TQ, 128)]
        t = jnp.concatenate([jnp.max(y.reshape(-1, 8, 128), axis=0) for y in parts], axis=1)
        return t if kc == 0 else jnp.maximum(mx, t)

    def row_max(mx):
        return jnp.broadcast_to(jnp.max(mx, axis=0, keepdims=True), (8, TQ))

    def grad_out(r, zero=0):
        return jnp.concatenate([doT[j + zero, r, :] for j in range(TQ // 128)], axis=1).astype(f32)

    def normed_x(b, r):
        return (xT[b, r, :].astype(f32) - ln1[b, 0, 0:1, :]) * ln1[b, 1, 0:1, :]

    def modulated_x(mod1, b, r):
        return (normed_x(b, r) * _wide(mod1[1, r, :]) + _wide(mod1[0, r, :])).astype(bf16)

    def prologue(x_v, wmod_v, wqT, mod1):
        wq = wo

        def x_copy(b):
            return copy(x_hbm.at[tokens(b)], x_v.at[b], 5 + b)

        cps = [copy(wq_hbm, wq, 0), copy(wkT_hbm, wkT, 1), copy(wvT_hbm, wvT, 2),
               copy(c_hbm, c_v, 3), copy(wmod_hbm.at[:, pl.ds(0, 2 * D)], wmod_v, 4)]
        for cp in [x_copy(b) for b in range(NB)] + cps[3:] + cps[:3] + [dout_copy(0)]:
            cp.start()

        for i in range(zeros.shape[0]):
            zeros[i] = 0

        def zero(i, carry):
            rows = pl.ds(pl.multiple_of(i * 64, 64), 64)
            dw1_acc[rows, :] = jnp.zeros((64, D), f32)
            dw2_acc[rows, :] = jnp.zeros((64, D), f32)
            return carry
        lax.fori_loop(0, F // 64, zero, 0)

        def statistics(b, carry):
            x_copy(b).wait()
            xT[b] = x_v[b].T
            mu, rstd = _layer_norm_stats(
                xT[b + zeros[0], r, :].astype(f32) for r in _chunks(D, DC))
            ln1[b, 0] = jnp.broadcast_to(mu, (8, TQ))
            ln1[b, 1] = jnp.broadcast_to(rstd, (8, TQ))
            ln1[b, 2] = jnp.zeros((8, TQ), f32)
            stat[b] = jnp.zeros((D, 128), f32)
            dkT[b] = jnp.zeros((W, TQ), f32)
            dvT[b] = jnp.zeros((W, TQ), f32)
            dwo_acc[pl.ds(pl.multiple_of(b * (D // NB), 8), D // NB), :] = jnp.zeros((D // NB, D), f32)
            return carry
        lax.fori_loop(0, NB, statistics, 0)

        for cp in cps[3:]:
            cp.wait()
        row = _nn(jnp.broadcast_to(silu_c()[0], (8, D)), wmod_v[...])
        set_modulation(mod1, row[0:1], 1)
        row_8 = lax.broadcasted_iota(jnp.int32, (8, D), 0)
        mod_rows[...] = jnp.where(row_8 == 0, 1.0, jnp.where(row_8 == 1, row[:, D:], row[:, :D]))

        for cp in cps[:3]:
            cp.wait()
        zpad = jnp.zeros((W - DH, D), f32)
        wqT[:2 * W, :] = jnp.concatenate(
            [wkT[...].astype(f32), zpad, wvT[...].astype(f32), zpad], axis=0).astype(bf16)
        wqT[2 * W:, :] = wq[...].T

        for b in range(NB):
            acc = None
            for r in _chunks(D, 128):
                acc = _accumulate(acc, _nn(wqT[:, r], modulated_x(mod1, b, r)))
            qT[b * D:(b + 1) * D, :] = (acc[2 * W:] * (SCALE * LOG2E)).astype(bf16)
            k_t = _round(acc[:W])
            v_t = jnp.where((row_w == DH) | (row_w == DH + 1), 1.0, _round(acc[W:2 * W]))
            kT[b] = k_t
            vT[b] = v_t
            fill = jnp.zeros((128 - W, TQ), f32)
            for src, keys, columns, groups in ((k_t, kk, k_cols, K_GROUPS),
                                               (v_t, va, v_cols, V_GROUPS)):
                rows = jnp.concatenate([src, fill], axis=0).T
                keys[b * TQ:(b + 1) * TQ, :] = rows[:, :WB]
                picked = jnp.concatenate([rows[at:at + 8] for at in groups], axis=0)
                for d in range(DH):
                    columns[b, d] = jnp.broadcast_to(picked[:, d:d + 1], columns.shape[2:])
            vT_swapped[b] = _swap_pairs(rows).T[:W]

        qs = [(_pad_rhs(q), _spread(q)) for q in _windows(qT[0:4 * DH, :].astype(f32))]
        mx = None
        for n in range(NC + LAG):
            u, kc = divmod(n, NC)
            mx = score_step(qs[u], kc, u, mx)
            if kc == NC - 1:
                m_buf[0] = row_max(mx)
        m_buf[1] = mx
        for cp in early_copies:
            cp.start()

    pl.run_scoped(prologue,
                  pltpu.VMEM((NB, TQ, D), bf16), pltpu.VMEM((D, 2 * D), bf16),
                  pltpu.VMEM((2 * W + D, D), bf16), pltpu.VMEM((2, D, 128), f32))

    def token_block(b, p_buf):
        def attn_fwd():
            dout_copy(b).wait()

            def body(i, carry):
                doT[i] = io_v[pl.ds(pl.multiple_of(i * 128, 128), 128), :].T
                h = b * H + i * HF
                qs = _windows(qT[head_rows(h, HF), :].astype(f32))
                qs += _windows(qT[head_rows(jnp.minimum(h + HF, NB * H - 4), 4), :].astype(f32))
                qs = [(_pad_rhs(q), _spread(q)) for q in qs]
                ms, seen, acc, outs = [m_buf[0]], [m_buf[1]], None, []

                def scores(n):
                    u, kc = divmod(n + NC + LAG, NC)
                    seen.append(score_step(qs[u], kc, u % 2, seen[-1]))
                    if kc == NC - 1:
                        ms.append(row_max(seen[-1]))

                for n in range(HF * NC):
                    if n + 1 < HF * NC:
                        scores(n)
                    u, kc = divmod(n, NC)
                    if n >= PACE:
                        ms[u] = jnp.maximum(ms[u], jnp.minimum(ms[u], seen[n + 1 - PACE]))
                    ks = slice(kc * KC, (kc + 1) * KC)
                    s = s_buf[u % 2, ks, :].reshape(KC // 8, 8, TQ)
                    p = jnp.exp2(s - ms[u][None]).reshape(KC, TQ)
                    p_buf[i * HF + u, ks, :] = p.astype(bf16)
                    t = _nn(key_tile(vT_swapped, kc)[...], _swap_pairs(p).astype(bf16))
                    acc = t if kc == 0 else acc + t
                    if kc == NC - 1:
                        inv = 1.0 / acc[DH:DH + 1]
                        o = acc * inv
                        ow[i * HF + u] = jnp.where(row_w == DH, inv, o)
                        outs.append(o[:DH])
                scores(HF * NC - 1)
                oT[head_rows(i * HF, HF), :] = jnp.concatenate(outs, axis=0).astype(bf16)
                m_buf[0] = ms[HF]
                m_buf[1] = seen[-1]
                return carry
            lax.fori_loop(0, H // HF, body, 0)

        def attn_bwd():
            def body(i, carry):
                @pl.when(i == 4)
                def _():
                    out_copy(b).wait()

                @pl.when(jnp.logical_and(i == 4, b + 1 < NB))
                def _():
                    dout_copy(b + 1).start()

                rows = head_rows(b * H + i * HU, HU)
                qs = _windows(qT[rows, :].astype(f32))
                rhs = [(_pad_rhs(w), _spread(w), w[DH:DH + 1] + w[DH + 1:DH + 2])
                       for w in (ow[i * HU + u] for u in range(HU))]

                def dscore(n):
                    u, kc = divmod(n, NC)
                    ks = slice(kc * KC, (kc + 1) * KC)
                    weights, spread, first = rhs[u]
                    for d in range(DH):
                        first = first + _wide(v_cols[kc // 4, d, kc % 4 * 8:kc % 4 * 8 + 8]) * spread[d]
                    dp = jnp.concatenate(
                        [first, _nn(va[kc * KC + 8:(kc + 1) * KC, :], weights)], axis=0)
                    return (p_buf[i * HU + u, ks, :].astype(f32) * dp).astype(bf16)

                def wo_grad(*tiles):
                    r = head_rows(i * HU, HU)
                    for t in tiles:
                        cols = slice(t * 128, (t + 1) * 128)
                        dwo_acc[r, cols] += _nt(oT[r, :], da[cols, :])

                ds_next, dq, dqs, q_dq = dscore(0), None, [], ln1[b, 2]
                wo_grad(0)
                for n in range(HU * NC):
                    ds = ds_next
                    if n + 1 < HU * NC:
                        ds_next = dscore(n + 1)
                    if n == 0:
                        wo_grad(1)
                    if n + 1 == HU * NC:
                        wo_grad(2, 3)
                    u, kc = divmod(n, NC)
                    ks = slice(kc * KC, (kc + 1) * KC)
                    key_tile(dvT, kc)[...] += _nt(ow[i * HU + u], p_buf[i * HU + u, ks, :])
                    if n + 1 < HU * NC:
                        key_tile(dkT, kc)[...] += _nt(qs[u], ds)
                    t = _nn(key_tile(kT, kc)[...], ds)
                    dq = t if kc == 0 else dq + t
                    if kc == NC - 1:
                        dqs.append(dq[:DH] * SCALE)
                        q_dq = q_dq + _rows8(qs[u] * dq)
                key_tile(dkT, kc)[...] += _nt(qs[u], ds)
                wo_grad(4)
                qT[rows, :] = jnp.concatenate(dqs, axis=0).astype(bf16)
                ln1[b, 2] = q_dq
                return carry
            lax.fori_loop(0, H // HU, body, 0)

        def dense():
            fcs = [(fs, slice(FH + fs.start, FH + fs.stop)) for fs in _chunks(FH, FC)]

            def work(k, r, slot=1):
                lo = LAG * TQ + k * D
                return s_buf.at[slot, pl.ds(lo + r.start, r.stop - r.start)]

            @pl.when(b == 0)
            def _():
                for cp in early_copies:
                    cp.wait()
                sc = jnp.broadcast_to(silu_c()[0], (8, D))
                w = jnp.concatenate([ref[...] for ref in mod_stage], axis=1)
                set_modulation(modc, _nn(sc, w)[0:1], SCALE_B)
                woT[...] = wo[...].T
                for src, dst in ((w1T, w1_left), (w2, w2_left)):
                    for k, lo in enumerate(range(0, FH, 128)):
                        n = min(128, FH - lo)
                        pad = [jnp.zeros((128 - n, D), bf16)] if n < 128 else []
                        near, far = (
                            jnp.concatenate([src[at:at + n, :]] + pad, axis=0).T.astype(f32)
                            for at in (lo, FH + lo))
                        for i, v in enumerate(_left_combinations(
                                near[:MH], far[:MH], near[MH:], far[MH:])):
                            dst[k, i * MH:(i + 1) * MH, :] = v.astype(bf16)

            def residual(r):
                a = _nn(woT[r, :], oT[...])
                work(0, r)[...] = a
                x1 = xT[b, r, :].astype(f32) + _wide(modc[GATE_A, r, :]) * a
                work(1, r)[...] = x1
                return x1

            mu, rstd = _layer_norm_stats(residual(r) for r in _chunks(D, DC))
            for r in _chunks(D, 128):
                dm[r, :] = (grad_out(r) * _wide(modc[GATE_B, r, :])).astype(bf16)
                h2[r, :] = ((work(1, r, 1 + zeros[1])[...] - mu) * rstd * _wide(modc[SCALE_B, r, :])
                            + _wide(modc[SHIFT_B, r, :])).astype(bf16)
            _store_sums(dm_sums, dm_buf.at[zeros[0]])
            _store_sums(h2_sums, h2_buf.at[zeros[0]])

            def weight_grads(fs):
                _add_weight_grad(dw2_acc, fs, g_buf, dm, dm_sums)
                _add_weight_grad(dw1_acc, fs, du_buf, h2, h2_sums)

            for i, pair in enumerate(fcs):
                gs, dus = [], []
                for fs in pair:
                    dg = _nn(w2[fs, :], dm[...])
                    uu = _nn(w1T[fs, :], h2[...])
                    sg = 0.5 * jnp.tanh(0.5 * uu) + 0.5
                    gg = uu * sg
                    du = dg * (sg + gg * (1.0 - sg))
                    gs += [gg[:, :TH], gg[:, TH:]]
                    dus += [du[:, :TH], du[:, TH:]]
                for dst, quads in ((g_buf, gs), (du_buf, dus)):
                    for n, v in enumerate(_left_combinations(*quads)):
                        dst[2 * n, pair[0], :] = v[:, :128].astype(bf16)
                        dst[2 * n + 1, pair[0], :] = v[:, 128:].astype(bf16)
                if i:
                    weight_grads(fcs[i - 1][0])
            weight_grads(fcs[-1][0])
            p1 = p2 = None
            for r, dh in _down_projection(w1_left, du_buf):
                ln = (work(1, r, 1 + zeros[2])[...] - mu) * rstd
                stat[SHIFT_B, r, :] += _fold(dh)
                stat[SCALE_B, r, :] += _fold(dh * ln)
                dl = dh * _wide(modc[SCALE_B, r, :])
                dm[r, :] = dl.astype(bf16)
                p1 = _accumulate(p1, _rows8(dl))
                p2 = _accumulate(p2, _rows8(dl * ln))
            c1, c2 = _mean_rows(p1), _mean_rows(p2)
            for r, mm in _down_projection(w2_left, g_buf):
                dy = grad_out(r, zeros[0])
                x1 = work(1, r, 1 + zeros[3])[...]
                stat[GATE_B, r, :] += _fold(dy * mm)
                ln = (x1 - mu) * rstd
                d1 = dy + rstd * (dm_buf[zeros[1], r, :].astype(f32) - c1 - ln * c2)
                dx1[b, r, :] = d1.astype(bf16)
                stat[GATE_A, r, :] += _fold(d1 * work(0, r, 1 + zeros[0])[...])
                da[r, :] = (d1 * _wide(modc[GATE_A, r, :])).astype(bf16)
                h2[r, :] = (x1 + _wide(modc[GATE_B, r, :]) * mm).astype(bf16)
            io_v[...] = h2[...].T

            for i, r in enumerate(_chunks(D, DC)):
                for u, do in enumerate(_windows(_nn(wo[r, :], da[...]))):
                    w = ow[i * (DC // DH) + u]
                    dwin = _round(do * w[DH:DH + 1])
                    delta = jnp.sum(dwin * w, axis=0, keepdims=True)
                    hi = _round(delta)
                    ow[i * (DC // DH) + u] = jnp.where(
                        row_w == DH, -hi, jnp.where(row_w == DH + 1, hi - delta, dwin))
            out_copy(b).start()

            @pl.when(b == NB - 1)
            def _():
                for i, (rows, t) in enumerate(grad_tiles):
                    du_buf[i] = dw1_acc[rows, t].astype(bf16)
                    g_buf[i] = dw2_acc[rows, t].astype(bf16)
                sc_col = _to_column(_round(silu_c()[0]))
                row = jnp.concatenate([_to_row(stat[j]) for j in range(4)], axis=1)
                dmod_v[:, 2 * D:] = jnp.broadcast_to(row, (8, 4 * D))
                for ref, t in zip(grad_stage, _chunks(4 * D, 128)):
                    ref[...] = (sc_col * row[:, t]).astype(bf16)
                for cp in [wq_copy] + grad_copies:
                    cp.start()

        attn_fwd()
        dense()
        attn_bwd()

    def epilogue(dwmod_v, dwq_v, dx_v, wkv, dkv, mean_w, sc_col, dc_parts, dkv_parts, dc_v,
                 stat1, mod1, wmod_v):
        wq = wo
        wmod_copy = copy(wmod_hbm, wmod_v, 23)
        wmod_copy.start()
        wq_copy.wait()
        set_modulation(mod1, jnp.concatenate([mod_rows[2:3, :], mod_rows[1:2, :]], axis=1), 1)

        def dx_copy(b):
            return copy(dx_v.at[b], dx_hbm.at[tokens(b)], b)

        def tile(i):
            return pl.ds(pl.multiple_of(i * 128, 128), 128)

        def dwq_copy(i):
            return copy(dwq_v.at[tile(i)], dwq_hbm.at[tile(i)], 4 + i)

        def dwmod_copy(i):
            return copy(dwmod_v.at[i], dwmod_hbm.at[tile(i), pl.ds(0, 2 * D)], 9 + i)

        def mod_weight_grad(i):
            for t in _chunks(2 * D, 128):
                dwmod_v[i, :, t] = (sc_col[tile(i), :] * dmod_v[0:1, t]).astype(bf16)

        zpad = jnp.zeros((W - DH, D), f32)
        wkv[...] = jnp.concatenate(
            [wkT[...].astype(f32), zpad, wvT[...].astype(f32),
             jnp.zeros((128 - W - DH, D), f32)], axis=0).T.astype(bf16)
        stat1[...] = jnp.zeros_like(stat1)
        woT[...] = dwo_acc[...].astype(bf16)
        dwo_copy = copy(woT, dwo_hbm, 24)
        sc_col[...] = _to_column(_round(silu_c()[0]))

        r = jnp.concatenate([_nn(mod_rows[...], wq[...]), _nn(mod_rows[...], wkv[...])], axis=1)
        row = lax.broadcasted_iota(jnp.int32, mean_w.shape, 0)
        mean_w[...] = jnp.where(row == 0, r[0:1] + r[1:2], r[2:3]).astype(bf16)

        dwo_copy.start()

        def input_grad(b, carry):
            dk = jnp.where(row_w < DH, dkT[b] * (1.0 / LOG2E), 0.0)
            dv = jnp.where(row_w < DH, dvT[b], 0.0)
            dkv[b] = jnp.concatenate([dk, dv], axis=0).astype(bf16)
            dot = ln1[b, 2] * (1.0 / LOG2E) + _rows8(kT[b] * dk + vT[b] * dv)
            dq = qT.at[pl.ds(pl.multiple_of(b * D, D), D)]
            for i, r in enumerate(_chunks(D, 128)):
                wq_r, wkv_r = wq[r, :], wkv[r, :2 * W]
                if i == 0:
                    wq_r = jnp.concatenate([mean_w[:, :D], wq_r], axis=0)
                    wkv_r = jnp.concatenate([mean_w[:, D:D + 2 * W], wkv_r], axis=0)
                dh = _nn(wq_r, dq[...]) + _nn(wkv_r, dkv[b])
                if i == 0:
                    c1 = dh[0:1] * (1.0 / D)
                    c2 = _mean_rows(dot) - dh[1:2] * (1.0 / D)
                    dh = dh[16:]
                ln = normed_x(b, r)
                stat1[0, r, :] += _fold(dh)
                stat1[1, r, :] += _fold(dh * ln)
                dx_v[b, :, r] = (dx1[b, r, :].astype(f32) + ln1[b, 1, 0:1, :]
                                 * (dh * _wide(mod1[1, r, :]) - c1 - ln * c2)).astype(bf16).T
            dx_copy(b).start()
            return carry
        lax.fori_loop(0, NB, input_grad, 0)

        wmod_copy.wait()
        for j in range(2):
            dmod_v[:, j * D:(j + 1) * D] = jnp.broadcast_to(_to_row(stat1[j]), (8, D))
        row = dmod_v[...]
        first = lax.broadcasted_iota(jnp.int32, row.shape, 0) == 0
        dmod_v[...] = jnp.where(first, row, row - _round(row))

        def weight_grad(i, carry):
            r = tile(i)
            dc_work = [slice(lo, min(lo + TQ, 6 * D)) for lo in range(0, 6 * D, TQ)]
            dwq = dwkv = dc = None
            for b in range(NB):
                h = modulated_x(mod1, b, r)
                parts = []
                for k, t in enumerate(_chunks(D, 128)):
                    parts.append(_nt(h, qT[b * D + t.start:b * D + t.stop, :]))
                    if k == 2:
                        dwkv = _accumulate(dwkv, _nt(dkv[b], h))
                    elif k in (0, 3):
                        cols = dc_work.pop()
                        dc = _accumulate(dc, _nt(dmod_v[:, cols], wmod_v[r, cols]))
                dwq = _accumulate(dwq, jnp.concatenate(parts, axis=1))
            assert not dc_work
            dwq_v[r, :] = dwq.astype(bf16)
            dkv_parts[i] = dwkv
            dc_parts[i] = dc
            mod_weight_grad(i)
            dwmod_copy(i).start()
            dwq_copy(i).start()
            return carry
        lax.fori_loop(0, D // 128, weight_grad, 0)

        dc = jnp.concatenate([dc_parts[i] for i in range(D // 128)], axis=1)
        dc_v[...] = ((dc[0:1] + dc[1:2]) * silu_c()[1]).astype(bf16)
        dwkv = jnp.concatenate([dkv_parts[i] for i in range(D // 128)], axis=1)
        wkT[...] = dwkv[:DH].astype(bf16)
        wvT[...] = dwkv[W:W + DH].astype(bf16)
        last = [copy(wkT, dwkT_hbm, 14), copy(wvT, dwvT_hbm, 15), copy(dc_v, dc_hbm, 16)]
        for cp in last:
            cp.start()

        for cp in grad_copies + [dwo_copy] + [dx_copy(b) for b in range(NB)]:
            cp.wait()
        for i in range(D // 128):
            dwmod_copy(i).wait()
            dwq_copy(i).wait()
        for cp in last:
            cp.wait()

    def block(b, carry):
        pl.run_scoped(functools.partial(token_block, b), pltpu.VMEM((H, S, TQ), bf16))

        @pl.when(b == NB - 1)
        def _():
            pl.run_scoped(
                epilogue,
                pltpu.VMEM((D // 128, 128, 2 * D), bf16), pltpu.VMEM((D, D), bf16),
                pltpu.VMEM((NB, TQ, D), bf16), pltpu.VMEM((D, 128), bf16),
                pltpu.VMEM((NB, 2 * W, TQ), bf16), pltpu.VMEM((16, D + 128), bf16),
                pltpu.VMEM((D, 128), f32), pltpu.VMEM((D // 128, 8, 128), f32),
                pltpu.VMEM((D // 128, 2 * W, 128), f32), pltpu.VMEM((1, D), bf16),
                pltpu.VMEM((2, D, 128), f32), pltpu.VMEM((2, D, 128), f32),
                pltpu.VMEM((D, 6 * D), bf16))
        return carry
    lax.fori_loop(0, NB, block, 0)


@jax.jit
def pallas_adaLN_cond__grouped_kv_mqa__dense_activation_silu__prompt_kernel(
    A_x: jax.Array,
    A_wq: jax.Array,
    A_wk: jax.Array,
    A_wv: jax.Array,
    A_wo: jax.Array,
    B_x: jax.Array,
    B_w1: jax.Array,
    B_w2: jax.Array,
    c: jax.Array,
    w_mod: jax.Array,
    grad_out: jax.Array,
):
    del B_x
    vm = pltpu.VMEM
    scratch = [
        vm((DH, D), bf16), vm((DH, D), bf16),
        vm((D, D), bf16), vm((D, D), bf16),
        vm((KT, 7 * MH, 128), bf16), vm((F, D), bf16),
        vm((F, D), bf16), vm((KT, 7 * MH, 128), bf16),
        vm((1, D), bf16),
        vm((4, D, 128), f32), vm((8, D), f32),
        vm((4, D, 128), f32), vm((NB, 3, 8, TQ), f32),
        vm((S, WB), f32), vm((S, WB), f32),
        vm((NB, DH, 8 * len(K_GROUPS), 128), f32),
        vm((NB, DH, 8 * len(V_GROUPS), 128), f32),
        *[vm((NB, W, TQ), f32)] * 5,
        vm((2, S, TQ), f32), vm((2, 8, TQ), f32),
        vm((H, W, TQ), f32), vm((TQ, D), bf16),
        vm((14, FH, 128), bf16), vm((14, FH, 128), bf16),
        vm((D, D), f32), vm((F, D), f32), vm((F, D), f32),
        vm((8, 6 * D), f32),
        pltpu.SMEM((4,), jnp.int32),
        pltpu.SemaphoreType.DMA((29,)),
    ]
    shapes = [(S, D), (S, D), (D, D), (DH, D), (DH, D), (D, D), (F, D), (F, D),
              (1, D), (D, 6 * D)]
    hbm = pl.BlockSpec(memory_space=pl.ANY)
    out, dx, dwq, dwkT, dwvT, dwo, dw1T, dw2, dc, dwmod = pl.pallas_call(
        _kernel,
        in_specs=[hbm] * 10,
        out_specs=[hbm] * 10,
        out_shape=[jax.ShapeDtypeStruct(s, bf16) for s in shapes],
        scratch_shapes=scratch,
        compiler_params=pltpu.CompilerParams(vmem_limit_bytes=128 * 2 ** 20),
        name="adaln_block",
    )(A_x.reshape(S, D), A_wq, A_wk.T, A_wv.T, A_wo, B_w1.T, B_w2, c, w_mod,
      grad_out.reshape(S, D))
    return (out.reshape(1, S, D), dx.reshape(1, S, D), dwq, dwkT.T, dwvT.T, dwo,
            dw1T.T, dw2, dc, dwmod)
```
